```python
import jax
import jax.numpy as jnp

def _softmax(x, axis=-1):
    return jax.nn.softmax(x, axis=axis)

def _gelu(x):
    return jax.nn.gelu(x, approximate=True)

def _silu(x):
    return jax.nn.silu(x)

def _sigmoid(x):
    return jax.nn.sigmoid(x)

def _layernorm(x, axis=-1, eps=1e-05):
    m = jnp.mean(x, axis=axis, keepdims=True)
    v = jnp.var(x, axis=axis, keepdims=True)
    return (x - m) / jnp.sqrt(v + eps)

def _scatter_add(tgt, idx, src, axis=0):
    return tgt.at[idx].add(src)

def _segment_sum(src, seg, n):
    return jax.ops.segment_sum(src, seg, n)

class _Rng:

    def __init__(self, key):
        self._k = key

    def _next(self):
        self._k, sub = jax.random.split(self._k)
        return sub

    def normal(self, shape):
        return jax.random.normal(self._next(), shape, dtype=jnp.bfloat16)

    def randint(self, lo, hi, shape):
        return jax.random.randint(self._next(), shape, lo, hi, dtype=jnp.int32)

    def uniform(self, shape, lo=0.0, hi=1.0):
        return jax.random.uniform(self._next(), shape, jnp.bfloat16, lo, hi)

    def permutation(self, n):
        return jax.random.permutation(self._next(), n)
kernel_name = 'adaLN_cond__compressed_kv_cla__mixer_s_mlp__prompt'

def setup_inputs():
    _rng = _Rng(jax.random.key(int.from_bytes(__import__("os").urandom(4), "little")))
    _w = lambda a: (lambda t: t.astype(jnp.bfloat16) if jnp.issubdtype(t.dtype, jnp.floating) else t)(jnp.asarray(a))

    def _A_setup():
        B, H, Sq, Sk, D, M = (1, 32, 2048, 2048, 128, 640)
        Dc = 4 * D
        return {'x': _w((lambda *s: _rng.normal(s) * 0.05)(B, Sq, M)), 'c_kv': _w((lambda *s: _rng.normal(s) * 0.05)(B, Sk, Dc)), 'w_q': _w((lambda *s: _rng.normal(s) * 0.05)(M, H, D) * M ** (-0.5)), 'w_uk': _w((lambda *s: _rng.normal(s) * 0.05)(Dc, H, D) * Dc ** (-0.5)), 'w_uv': _w((lambda *s: _rng.normal(s) * 0.05)(Dc, H, D) * Dc ** (-0.5)), 'w_o': _w((lambda *s: _rng.normal(s) * 0.05)(H, D, M) * (H * D) ** (-0.5))}
    _A_in = _A_setup()

    def _B_setup():
        B, S, D, F = (1, 2048, 640, 1728)
        return {'x': _w((lambda *s: _rng.normal(s) * 0.05)(B, S, D)), 'w1': _w((lambda *s: _rng.normal(s) * 0.05)(D, D) * D ** (-0.5)), 'w2': _w((lambda *s: _rng.normal(s) * 0.05)(D, D) * D ** (-0.5)), 'w3': _w((lambda *s: _rng.normal(s) * 0.05)(D, F) * D ** (-0.5)), 'w4': _w((lambda *s: _rng.normal(s) * 0.05)(F, D) * F ** (-0.5))}
    _B_in = _B_setup()
    return {'A_x': _A_in['x'], 'A_c_kv': _A_in['c_kv'], 'A_w_q': _A_in['w_q'], 'A_w_uk': _A_in['w_uk'], 'A_w_uv': _A_in['w_uv'], 'A_w_o': _A_in['w_o'], 'B_x': _B_in['x'], 'B_w1': _B_in['w1'], 'B_w2': _B_in['w2'], 'B_w3': _B_in['w3'], 'B_w4': _B_in['w4'], 'c': _w((lambda *s: _rng.normal(s) * 0.05)(1, 640)), 'w_mod': _w((lambda *s: _rng.normal(s) * 0.05)(640, 6 * 640) * 640 ** (-0.5))}

def reference(A_x, A_c_kv, A_w_q, A_w_uk, A_w_uv, A_w_o, B_x, B_w1, B_w2, B_w3, B_w4, c, w_mod):

    def _A_ref(x, c_kv, w_q, w_uk, w_uv, w_o):
        B, Sq, M = (x.shape[0], x.shape[1], x.shape[2])
        Sk = c_kv.shape[1]
        H, D = (w_q.shape[1], w_q.shape[2])
        q = jnp.einsum('bqm,mhd->bhqd', x, w_q)
        k = jnp.einsum('bkc,chd->bhkd', c_kv, w_uk)
        v = jnp.einsum('bkc,chd->bhkd', c_kv, w_uv)
        scores = jnp.einsum('bhqd,bhkd->bhqk', q, k) * D ** (-0.5)
        off = Sk - Sq
        qi = jnp.arange(Sq)[:, None]
        kj = jnp.arange(Sk)[None, :]
        cmask = kj <= qi + off
        scores = jnp.where(cmask[None, None], scores, -1000000000.0)
        p = _softmax(scores, axis=-1)
        ctx = jnp.einsum('bhqk,bhkd->bhqd', p, v)
        return jnp.einsum('bhqd,hdm->bqm', ctx, w_o)

    def _B_ref(x, w1, w2, w3, w4):
        B, S, D = x.shape
        h = _gelu(_layernorm(x, axis=-1) @ w1)
        c = D // 4
        g0 = jnp.pad(h[:, :, 0 * c:1 * c], ((0, 0), (1, 0), (0, 0)))[:, :S, :]
        g1 = jnp.pad(h[:, :, 1 * c:2 * c], ((0, 0), (0, 1), (0, 0)))[:, 1:, :]
        g2 = jnp.pad(h[:, :, 2 * c:3 * c], ((0, 0), (2, 0), (0, 0)))[:, :S, :]
        g3 = jnp.pad(h[:, :, 3 * c:], ((0, 0), (0, 2), (0, 0)))[:, 2:, :]
        hs = jnp.concatenate([g0, g1, g2, g3], axis=-1) @ w2
        x1 = x + hs
        h2 = _gelu(_layernorm(x1, axis=-1) @ w3) @ w4
        return x1 + h2
    x = A_x
    mod = (_silu(c) @ w_mod).reshape(c.shape[0], 6, 1, -1)
    sa, ca, ga, sb, cb, gb = (mod[:, 0].copy(), mod[:, 1].copy(), mod[:, 2].copy(), mod[:, 3].copy(), mod[:, 4].copy(), mod[:, 5].copy())
    h = _layernorm(x, axis=-1) * (1 + ca) + sa
    x = x + ga * _A_ref(h, A_c_kv, A_w_q, A_w_uk, A_w_uv, A_w_o)
    h = _layernorm(x, axis=-1) * (1 + cb) + sb
    x = x + gb * _B_ref(h, B_w1, B_w2, B_w3, B_w4)
    return x
```

```python
import functools
import jax
import jax.numpy as jnp
import numpy as np
from jax.experimental import pallas as pl
from jax.experimental.pallas import tpu as pltpu

S = 2048; M = 640; H = 32; D = 128; DC = 512; F = 1728
NP = H // 2
NT = (((1,), (1,)), ((), ()))
LOG2E = 1.4426950408889634
NEG = -1e30
f32 = jnp.float32; bf16 = jnp.bfloat16; u32 = jnp.uint32


def _ln(x):
    m = jnp.mean(x, axis=-1, keepdims=True)
    xc = x - m
    v = jnp.mean(xc * xc, axis=-1, keepdims=True)
    return xc * jax.lax.rsqrt(v + 1e-5)


def _gelu(x):
    return 0.5 * x * (1.0 + jnp.tanh(0.7978845608028654 * (x + 0.044715 * (x * x * x))))


def _unpack_pair(w):
    lo = pltpu.bitcast(w << 16, f32).astype(bf16)
    hi = pltpu.bitcast(w & np.uint32(0xFFFF0000), f32).astype(bf16)
    return jnp.concatenate([lo, hi], axis=1)


def _finish(o, l):
    rl = pl.reciprocal(l, approx=True)
    rl = rl * (2.0 - l * rl)
    return (o * rl).astype(bf16)


def attn_blocks(q, k, v, BQ, order, DS, mode):
    outs = {}
    r = jax.lax.broadcasted_iota(jnp.int32, (DS, DS), 0)
    c = jax.lax.broadcasted_iota(jnp.int32, (DS, DS), 1)
    mask = c <= r
    dot = lambda a, b: jnp.dot(a, b, preferred_element_type=f32)
    dnt = lambda a, b: jax.lax.dot_general(a, b, NT, preferred_element_type=f32)
    for i in order:
        qi = q[i * BQ:(i + 1) * BQ]
        o0 = i * BQ
        if i > 0:
            s_off = dnt(qi, k[:o0])
        n = BQ // DS
        if mode == "row":
            ms, ss = [], []
            for rr in range(n):
                s = dnt(qi[rr * DS:(rr + 1) * DS], k[o0:o0 + (rr + 1) * DS])
                last = jnp.where(mask, s[:, rr * DS:], NEG)
                s = jnp.concatenate([s[:, :rr * DS], last], 1) if rr > 0 else last
                m = jnp.max(s, axis=1, keepdims=True)
                ms.append(m); ss.append(s)
            m = jnp.concatenate(ms, 0) if n > 1 else ms[0]
            if i > 0:
                m = jnp.maximum(m, jnp.max(s_off, axis=1, keepdims=True))
            ls, os_ = [], []
            for rr in range(n):
                p = jnp.exp2(ss[rr] - m[rr * DS:(rr + 1) * DS])
                ls.append(jnp.sum(p, axis=1, keepdims=True))
                os_.append(dot(p.astype(bf16), v[o0:o0 + (rr + 1) * DS]))
            l = jnp.concatenate(ls, 0) if n > 1 else ls[0]
            o = jnp.concatenate(os_, 0) if n > 1 else os_[0]
            if i > 0:
                p = jnp.exp2(s_off - m)
                l = l + jnp.sum(p, axis=1, keepdims=True)
                o = o + dot(p.astype(bf16), v[:o0])
            outs[i] = _finish(o, l)
        elif mode == "col":
            sd = []
            for jj in range(n):
                s = dnt(qi[jj * DS:], k[o0 + jj * DS:o0 + (jj + 1) * DS])
                top = jnp.where(mask, s[:DS], NEG)
                s = jnp.concatenate([top, s[DS:]], 0) if jj < n - 1 else top
                sd.append(s)
            ms = []
            for rr in range(n):
                m = functools.reduce(jnp.maximum, [sd[jj][(rr - jj) * DS:(rr - jj + 1) * DS] for jj in range(rr + 1)])
                if i > 0:
                    m = jnp.maximum(jnp.max(m, axis=1, keepdims=True), jnp.max(s_off[rr * DS:(rr + 1) * DS], axis=1, keepdims=True))
                else:
                    m = jnp.max(m, axis=1, keepdims=True)
                ms.append(m)
            m = jnp.concatenate(ms, 0) if n > 1 else ms[0]
            lr = [None] * n; orr = [None] * n
            if i > 0:
                p = jnp.exp2(s_off - m)
                l = jnp.sum(p, axis=1, keepdims=True)
                o = dot(p.astype(bf16), v[:o0])
                for rr in range(n):
                    lr[rr] = l[rr * DS:(rr + 1) * DS]; orr[rr] = o[rr * DS:(rr + 1) * DS]
            for jj in range(n):
                pj = jnp.exp2(sd[jj] - m[jj * DS:])
                lj = jnp.sum(pj, axis=1, keepdims=True)
                oj = dot(pj.astype(bf16), v[o0 + jj * DS:o0 + (jj + 1) * DS])
                for rr in range(jj, n):
                    a_, b_ = lj[(rr - jj) * DS:(rr - jj + 1) * DS], oj[(rr - jj) * DS:(rr - jj + 1) * DS]
                    lr[rr] = a_ if lr[rr] is None else lr[rr] + a_
                    orr[rr] = b_ if orr[rr] is None else orr[rr] + b_
            outs[i] = jnp.concatenate([_finish(orr[rr], lr[rr]) for rr in range(n)], 0) if n > 1 else _finish(orr[0], lr[0])
    return jnp.concatenate([outs[i] for i in range(S // BQ)], axis=0)


def attn_pair_sched(q2, k2, v2, BQ, la, inter, rev, diag_last, out_fn=None, OB=1):
    r = jax.lax.broadcasted_iota(jnp.int32, (BQ, BQ), 0)
    c = jax.lax.broadcasted_iota(jnp.int32, (BQ, BQ), 1)
    mask = c <= r
    dot = lambda a, b: jnp.dot(a, b, preferred_element_type=f32)
    dnt = lambda a, b: jax.lax.dot_general(a, b, NT, preferred_element_type=f32)
    nb = S // BQ
    blocks = list(range(nb))[::-1] if rev else list(range(nb))
    if inter:
        units = [(g, i) for i in blocks for g in range(2)]
    else:
        units = [(g, i) for g in range(2) for i in blocks]
    st = {}

    def A(u):
        g, i = u
        q = q2[i * BQ:(i + 1) * BQ, g * D:(g + 1) * D]
        k = k2[:, g * D:(g + 1) * D]
        o0 = i * BQ
        if diag_last:
            s_off = dnt(q, k[:o0]) if i > 0 else None
            s_d = dnt(q, k[o0:o0 + BQ])
        else:
            s_d = dnt(q, k[o0:o0 + BQ])
            s_off = dnt(q, k[:o0]) if i > 0 else None
        st[u] = (s_off, s_d)

    def B(u):
        g, i = u
        s_off, s_d = st[u]
        s_d = jnp.where(mask, s_d, NEG)
        m = jnp.max(s_d, axis=1, keepdims=True)
        if i > 0:
            m = jnp.maximum(m, jnp.max(s_off, axis=1, keepdims=True))
        p_d = jnp.exp2(s_d - m)
        l = jnp.sum(p_d, axis=1, keepdims=True)
        p = None
        if i > 0:
            p = jnp.exp2(s_off - m)
            l = l + jnp.sum(p, axis=1, keepdims=True)
            p = p.astype(bf16)
        st[u] = (p, p_d.astype(bf16), l)

    def C(u):
        g, i = u
        p, p_d, l = st[u]
        v = v2[:, g * D:(g + 1) * D]
        o0 = i * BQ
        o = dot(p_d, v[o0:o0 + BQ])
        if i > 0:
            o = o + dot(p, v[:o0])
        st[u] = _finish(o, l)

    n = len(units)
    done = set(); emitted = set()
    for t in range(n + la):
        if t < n:
            A(units[t])
        if t - la >= 0:
            B(units[t - la])
            C(units[t - la])
            if out_fn is not None:
                done.add(units[t - la])
                for ib in range(nb // OB):
                    need = [(g, i) for g in range(2) for i in range(ib * OB, (ib + 1) * OB)]
                    if ib not in emitted and all(u in done for u in need):
                        emitted.add(ib)
                        cc = jnp.concatenate([jnp.concatenate([st[(g, i)] for i in range(ib * OB, (ib + 1) * OB)], 0) if OB > 1 else st[(g, ib)] for g in range(2)], 1)
                        out_fn(ib * OB * BQ, OB * BQ, cc)
    if out_fn is not None:
        return None
    return jnp.concatenate([jnp.concatenate([st[(g, i)] for i in range(nb)], 0) for g in range(2)], 1)


def kernel(x_hbm, ckv_hbm, wq_hbm, wuk_hbm, wuv_hbm, wo_hbm, w1_hbm, w2_hbm, w3_hbm, w4_hbm, c_ref, wmod_hbm,
           o_ref,
           x_s, ckv_s, wq_b, wuk_b, wuv_b, wo_b, w1_s, w2_s, w3_s, w4_s, wmod_s,
           h_s, mod_s, acc_s, h1_s, sem, wsem, *, BQ, RB, order, NP, skipB, loopB, DS, mode, sched):
    p = pl.program_id(0)
    wq32 = wq_hbm.bitcast(u32)
    wuk32 = wuk_hbm.bitcast(u32)
    wuv32 = wuv_hbm.bitcast(u32)

    def wcopies(pp, slot):
        return [
            pltpu.make_async_copy(wuk32.at[:, pp, :], wuk_b.at[slot], wsem.at[slot, 0]),
            pltpu.make_async_copy(wuv32.at[:, pp, :], wuv_b.at[slot], wsem.at[slot, 1]),
            pltpu.make_async_copy(wq32.at[:, pp, :], wq_b.at[slot], wsem.at[slot, 2]),
            pltpu.make_async_copy(wo_hbm.at[pl.ds(pp * 2 * D, 2 * D), :], wo_b.at[slot], wsem.at[slot, 3]),
        ]

    cp_ckv = pltpu.make_async_copy(ckv_hbm, ckv_s, sem.at[0])
    cp_x = pltpu.make_async_copy(x_hbm, x_s, sem.at[1])
    cp_mod1 = pltpu.make_async_copy(wmod_hbm.at[:, 0:2 * M], wmod_s.at[:, 0:2 * M], sem.at[2])
    cp_mod2 = pltpu.make_async_copy(wmod_hbm.at[:, 2 * M:6 * M], wmod_s.at[:, 2 * M:6 * M], sem.at[3])
    cp_w1 = pltpu.make_async_copy(w1_hbm, w1_s, sem.at[4])
    cp_w2 = pltpu.make_async_copy(w2_hbm, w2_s, sem.at[5])
    cp_w3 = pltpu.make_async_copy(w3_hbm, w3_s, sem.at[6])
    cp_w4 = pltpu.make_async_copy(w4_hbm, w4_s, sem.at[7])

    @pl.when(p == 0)
    def _():
        first = wcopies(0, 0)
        cp_ckv.start()
        first[0].start()
        first[1].start()
        cp_mod1.start()
        cp_x.start()
        first[2].start()
        first[3].start()
        for cp in (cp_mod2, cp_w1, cp_w2, cp_w3, cp_w4):
            cp.start()
        cc = c_ref[...].astype(f32)
        sc = jnp.broadcast_to(cc * jax.nn.sigmoid(cc), (8, M)).astype(bf16)
        cp_mod1.wait()
        mod = jnp.dot(sc, wmod_s[:, 0:2 * M], preferred_element_type=f32)
        sa = mod[0:1, 0:M]
        ca1 = 1.0 + mod[0:1, M:2 * M]
        cp_x.wait()
        for r in range(S // RB):
            xr = x_s[r * RB:(r + 1) * RB, :].astype(f32)
            h_s[r * RB:(r + 1) * RB, :] = (_ln(xr) * ca1 + sa).astype(bf16)
        acc_s[...] = jnp.zeros_like(acc_s)
        cp_ckv.wait()

    slot = p % 2

    @pl.when(p + 1 < NP)
    def _():
        for cp in wcopies(p + 1, 1 - slot):
            cp.start()

    for cp in wcopies(p, slot):
        cp.wait()

    wuk = _unpack_pair(wuk_b[slot])
    wq = _unpack_pair(wq_b[slot])
    wuv = _unpack_pair(wuv_b[slot])
    h = h_s[...]
    ckv = ckv_s[...]
    k2 = jnp.dot(ckv, wuk, preferred_element_type=f32).astype(bf16)
    q2 = (jnp.dot(h, wq, preferred_element_type=f32) * (D ** -0.5 * LOG2E)).astype(bf16)
    v2 = jnp.dot(ckv, wuv, preferred_element_type=f32).astype(bf16)
    if sched is None:
        ctx = [attn_blocks(q2[:, g * D:(g + 1) * D], k2[:, g * D:(g + 1) * D], v2[:, g * D:(g + 1) * D], BQ, order, DS, mode)
               for g in range(2)]
        ctx2 = jnp.concatenate(ctx, axis=1)
        acc_s[...] += jnp.dot(ctx2, wo_b[slot], preferred_element_type=f32)
    elif len(sched) == 4:
        ctx2 = attn_pair_sched(q2, k2, v2, BQ, *sched)
        acc_s[...] += jnp.dot(ctx2, wo_b[slot], preferred_element_type=f32)
    else:
        wo = wo_b[slot]
        def out_fn(r0, n, cc):
            acc_s[r0:r0 + n, :] += jnp.dot(cc, wo, preferred_element_type=f32)
        attn_pair_sched(q2, k2, v2, BQ, *sched[:4], out_fn, sched[4])

    @pl.when(p == NP - 1)
    def _():
        if skipB:
            for cp in (cp_mod2, cp_w1, cp_w2, cp_w3, cp_w4): cp.wait()
            o_ref[...] = acc_s[...].astype(bf16)
            return
        cc = c_ref[...].astype(f32)
        sc = jnp.broadcast_to(cc * jax.nn.sigmoid(cc), (8, M)).astype(bf16)
        cp_mod2.wait()
        mod = jnp.dot(sc, wmod_s[:, 2 * M:6 * M], preferred_element_type=f32)
        ga = mod[0:1, 0:M]
        sb = mod[0:1, M:2 * M]
        cb1 = 1.0 + mod[0:1, 2 * M:3 * M]
        gb = mod[0:1, 3 * M:4 * M]
        cp_w1.wait()
        h1_s[0:8, :] = jnp.zeros((8, M), f32)
        h1_s[S + 8:S + 16, :] = jnp.zeros((8, M), f32)
        def stage1(r, carry):
            r0 = pl.multiple_of(r * RB, RB)
            rows = pl.ds(r0, RB)
            xm = x_s[rows, :].astype(f32) + ga * acc_s[rows, :]
            hb = _ln(xm) * cb1 + sb
            acc_s[rows, :] = hb
            t = jnp.dot(_ln(hb).astype(bf16), w1_s[...], preferred_element_type=f32)
            h1_s[pl.ds(r0 + 8, RB), :] = _gelu(t)
            x_s[rows, :] = xm.astype(bf16)
            return carry
        if loopB:
            jax.lax.fori_loop(0, S // RB, stage1, 0)
        else:
            for r in range(S // RB): stage1(r, 0)
        cp_w2.wait()
        cp_w3.wait()
        cp_w4.wait()
        c128 = jax.lax.broadcasted_iota(jnp.int32, (RB, 128), 1)
        def stage2(r, carry):
            r0 = pl.multiple_of(r * RB, RB)
            rows = pl.ds(r0, RB)
            hh = h1_s[pl.ds(r0, RB + 16), :]
            g0 = hh[7:7 + RB, 0:256]
            g1 = hh[9:9 + RB, 128:384]
            g2 = hh[6:6 + RB, 256:512]
            g3 = hh[10:10 + RB, 384:640]
            G = jnp.concatenate([
                g0[:, 0:128],
                jnp.where(c128 < 32, g0[:, 128:256], g1[:, 0:128]),
                jnp.where(c128 < 64, g1[:, 128:256], g2[:, 0:128]),
                jnp.where(c128 < 96, g2[:, 128:256], g3[:, 0:128]),
                g3[:, 128:256],
            ], axis=1).astype(bf16)
            hs = jnp.dot(G, w2_s[...], preferred_element_type=f32)
            x1 = acc_s[rows, :] + hs
            t = jax.lax.dot_general(_ln(x1).astype(bf16), w3_s[...], NT, preferred_element_type=f32)
            h2 = jnp.dot(_gelu(t).astype(bf16), w4_s[...], preferred_element_type=f32)
            o_ref[rows, :] = (x_s[rows, :].astype(f32) + gb * (x1 + h2)).astype(o_ref.dtype)
            return carry
        if loopB:
            jax.lax.fori_loop(0, S // RB, stage2, 0)
        else:
            for r in range(S // RB): stage2(r, 0)


def make(BQ=128, RB=256, vmem=110, flags=None, order=None, NP=16, skipB=False, loopB=True, DS=None, mode='row', sched=(1, 1, 0, True, 4)):
    DS = DS or BQ
    if order is None:
        order = list(range(S // BQ))[::-1]
    def run(A_x, A_c_kv, A_w_q, A_w_uk, A_w_uv, A_w_o, B_x, B_w1, B_w2, B_w3, B_w4, c, w_mod):
        x = A_x.reshape(S, M)
        ckv = A_c_kv.reshape(S, DC)
        wo = A_w_o.reshape(H * D, M)
        hbm = pl.BlockSpec(memory_space=pl.ANY)
        in_specs = [hbm] * 10 + [pl.BlockSpec((1, M), lambda p: (0, 0)), hbm]
        out = pl.pallas_call(
            functools.partial(kernel, BQ=BQ, RB=RB, order=order, NP=NP, skipB=skipB, loopB=loopB, DS=DS, mode=mode, sched=sched),
            grid=(NP,),
            in_specs=in_specs,
            out_specs=pl.BlockSpec((S, M), lambda p: (0, 0), pipeline_mode=pl.Buffered(1)),
            out_shape=jax.ShapeDtypeStruct((S, M), bf16),
            scratch_shapes=[
                pltpu.VMEM((S, M), bf16),
                pltpu.VMEM((S, DC), bf16),
                pltpu.VMEM((2, M, D), u32),
                pltpu.VMEM((2, DC, D), u32),
                pltpu.VMEM((2, DC, D), u32),
                pltpu.VMEM((2, 2 * D, M), bf16),
                pltpu.VMEM((M, M), bf16), pltpu.VMEM((M, M), bf16), pltpu.VMEM((F, M), bf16), pltpu.VMEM((F, M), bf16),
                pltpu.VMEM((M, 6 * M), bf16),
                pltpu.VMEM((S, M), bf16),
                pltpu.VMEM((8, 6 * M), f32),
                pltpu.VMEM((S, M), f32),
                pltpu.VMEM((S + 16, M), f32),
                pltpu.SemaphoreType.DMA((8,)),
                pltpu.SemaphoreType.DMA((2, 4)),
            ],
            compiler_params=pltpu.CompilerParams(
                dimension_semantics=("arbitrary",), vmem_limit_bytes=vmem * 1024 * 1024, flags=flags or {}),
        )(x, ckv, A_w_q, A_w_uk, A_w_uv, wo, B_w1, B_w2, B_w3.T, B_w4, c, w_mod)
        return out.reshape(1, S, M)
    return jax.jit(run)


def abstract_args():
    sd = jax.ShapeDtypeStruct
    return (sd((1, S, M), bf16), sd((1, S, DC), bf16), sd((M, H, D), bf16), sd((DC, H, D), bf16), sd((DC, H, D), bf16),
            sd((H, D, M), bf16), sd((1, S, M), bf16), sd((M, M), bf16), sd((M, M), bf16), sd((M, F), bf16),
            sd((F, M), bf16), sd((1, M), bf16), sd((M, 6 * M), bf16))


@jax.jit
def pallas_adaLN_cond__compressed_kv_cla__mixer_s_mlp__prompt_kernel(
    A_x, A_c_kv, A_w_q, A_w_uk, A_w_uv, A_w_o, B_x, B_w1, B_w2, B_w3, B_w4, c, w_mod):
    return make()(A_x, A_c_kv, A_w_q, A_w_uk, A_w_uv, A_w_o, B_x, B_w1, B_w2, B_w3, B_w4, c, w_mod)
```

```python
import functools

import jax
import jax.numpy as jnp
import numpy as np
from jax.experimental import pallas as pl
from jax.experimental.pallas import tpu as pltpu

S = 2048
M = 640
H = 32
D = 128
DC = 512
F = 1728
NP = H // 2
BQ = 128
RB = 256
EPS = 1e-5
NT = (((1,), (1,)), ((), ()))
LOG2E = 1.4426950408889634
NEG = -1e30
f32 = jnp.float32
bf16 = jnp.bfloat16
u32 = jnp.uint32

BLOCK_ORDER = (10, 1, 14, 7, 3, 5, 15, 0, 13, 6, 11, 8, 4, 12, 2, 9)
LOOKAHEAD = 1


def _dot(a, b):
    return jnp.dot(a, b, preferred_element_type=f32)


def _dot_nt(a, b):
    return jax.lax.dot_general(a, b, NT, preferred_element_type=f32)


def _ln(x):
    mean = jnp.mean(x, axis=-1, keepdims=True)
    xc = x - mean
    var = jnp.mean(xc * xc, axis=-1, keepdims=True)
    return xc * jax.lax.rsqrt(var + EPS)


def _gelu(x):
    return 0.5 * x * (1.0 + jnp.tanh(0.7978845608028654 * (x + 0.044715 * (x * x * x))))


def _unpack_pair(w):
    lo = pltpu.bitcast(w << 16, f32).astype(bf16)
    hi = pltpu.bitcast(w & np.uint32(0xFFFF0000), f32).astype(bf16)
    return jnp.concatenate([lo, hi], axis=1)


def _attention_step(h, ckv, wq, wuk, wuv, store_ctx):
    k2 = _dot(ckv, wuk).astype(bf16)
    q2 = (_dot(h, wq) * (D ** -0.5 * LOG2E)).astype(bf16)
    v2 = _dot(ckv, wuv).astype(bf16)
    row = jax.lax.broadcasted_iota(jnp.int32, (BQ, BQ), 0)
    col = jax.lax.broadcasted_iota(jnp.int32, (BQ, BQ), 1)
    causal = col <= row
    units = [(g, i) for i in BLOCK_ORDER for g in range(2)]
    scores = {}

    def qk(u):
        g, i = u
        q = q2[i * BQ:(i + 1) * BQ, g * D:(g + 1) * D]
        k = k2[:, g * D:(g + 1) * D]
        s_off = _dot_nt(q, k[:i * BQ]) if i > 0 else None
        scores[u] = (s_off, _dot_nt(q, k[i * BQ:(i + 1) * BQ]))

    def softmax_pv(u):
        g, i = u
        s_off, s_d = scores.pop(u)
        v = v2[:, g * D:(g + 1) * D]
        s_d = jnp.where(causal, s_d, NEG)
        m = jnp.max(s_d, axis=1, keepdims=True)
        if i > 0:
            m = jnp.maximum(m, jnp.max(s_off, axis=1, keepdims=True))
        p_d = jnp.exp2(s_d - m)
        l = jnp.sum(p_d, axis=1, keepdims=True)
        if i > 0:
            p_off = jnp.exp2(s_off - m)
            l = l + jnp.sum(p_off, axis=1, keepdims=True)
            p_off = p_off.astype(bf16)
        o = _dot(p_d.astype(bf16), v[i * BQ:(i + 1) * BQ])
        if i > 0:
            o = o + _dot(p_off, v[:i * BQ])
        r = pl.reciprocal(l, approx=True)
        r = r * (2.0 - l * r)
        store_ctx(g, i, (o * r).astype(bf16))

    issued = 0
    for t, u in enumerate(units):
        while issued < len(units) and issued <= t + LOOKAHEAD:
            qk(units[issued])
            issued += 1
        softmax_pv(u)


def _kernel(x_hbm, ckv_hbm, wq_hbm, wuk_hbm, wuv_hbm, wo_hbm, w1_hbm, w2_hbm, w3t_hbm, w4_hbm, c_ref, wmod_hbm,
            o_hbm,
            x_s, ckv_s, wq_b, wuk_b, wuv_b, wo_s, w1_s, w2_s, w3t_s, w4_s, wmod_s,
            h_s, ctx_s, hb_s, h1_s, sem, wsem, osem):
    p = pl.program_id(0)
    wq32 = wq_hbm.bitcast(u32)
    wuk32 = wuk_hbm.bitcast(u32)
    wuv32 = wuv_hbm.bitcast(u32)

    def pair_copies(pp, slot):
        return [pltpu.make_async_copy(wuk32.at[:, pp, :], wuk_b.at[slot], wsem.at[slot, 0]),
                pltpu.make_async_copy(wuv32.at[:, pp, :], wuv_b.at[slot], wsem.at[slot, 1]),
                pltpu.make_async_copy(wq32.at[:, pp, :], wq_b.at[slot], wsem.at[slot, 2])]

    cp_mod1 = pltpu.make_async_copy(wmod_hbm.at[:, 0:2 * M], wmod_s.at[:, 0:2 * M], sem.at[0])
    cp_x = pltpu.make_async_copy(x_hbm, x_s, sem.at[1])
    cp_ckv = pltpu.make_async_copy(ckv_hbm, ckv_s, sem.at[2])
    cp_wo = pltpu.make_async_copy(wo_hbm, wo_s, sem.at[3])
    cp_mod2 = pltpu.make_async_copy(wmod_hbm.at[:, 2 * M:6 * M], wmod_s.at[:, 2 * M:6 * M], sem.at[4])
    cp_w1 = pltpu.make_async_copy(w1_hbm, w1_s, sem.at[5])
    cp_w2 = pltpu.make_async_copy(w2_hbm, w2_s, sem.at[6])
    cp_w3 = pltpu.make_async_copy(w3t_hbm, w3t_s, sem.at[7])
    cp_w4 = pltpu.make_async_copy(w4_hbm, w4_s, sem.at[8])

    def silu_c():
        cc = c_ref[...].astype(f32)
        return jnp.broadcast_to(cc * jax.nn.sigmoid(cc), (8, M)).astype(bf16)

    @pl.when(p == 0)
    def _prologue():
        for cp in [cp_mod1, cp_x, cp_ckv] + pair_copies(0, 0):
            cp.start()
        sc = silu_c()
        cp_mod1.wait()
        mod = _dot(sc, wmod_s[:, 0:2 * M])
        sa = mod[0:1, 0:M]
        ca1 = 1.0 + mod[0:1, M:2 * M]
        cp_x.wait()

        def ln_chunk(r, carry):
            rows = pl.ds(pl.multiple_of(r * RB, RB), RB)
            h_s[rows, :] = (_ln(x_s[rows, :].astype(f32)) * ca1 + sa).astype(bf16)
            return carry
        jax.lax.fori_loop(0, S // RB, ln_chunk, 0)
        cp_ckv.wait()
        for cp in (cp_wo, cp_mod2, cp_w1, cp_w2, cp_w3, cp_w4):
            cp.start()

    slot = p % 2

    @pl.when(p + 1 < NP)
    def _prefetch():
        for cp in pair_copies(p + 1, 1 - slot):
            cp.start()

    for cp in pair_copies(p, slot):
        cp.wait()

    def store_ctx(g, i, val):
        ctx_s[p, i * BQ:(i + 1) * BQ, g * D:(g + 1) * D] = val

    _attention_step(h_s[...], ckv_s[...], _unpack_pair(wq_b[slot]), _unpack_pair(wuk_b[slot]),
                    _unpack_pair(wuv_b[slot]), store_ctx)

    @pl.when(p == NP - 1)
    def _mixer():
        cp_mod2.wait()
        mod = _dot(silu_c(), wmod_s[:, 2 * M:6 * M])
        ga = mod[0:1, 0:M]
        sb = mod[0:1, M:2 * M]
        cb1 = 1.0 + mod[0:1, 2 * M:3 * M]
        gb = mod[0:1, 3 * M:4 * M]
        cp_wo.wait()
        cp_w1.wait()
        h1_s[0:8, :] = jnp.zeros((8, M), f32)
        h1_s[S + 8:S + 16, :] = jnp.zeros((8, M), f32)

        def stage1(r, carry):
            r0 = pl.multiple_of(r * RB, RB)
            n = RB // 4
            att = []
            for j in range(4):
                rows = pl.ds(r0 + j * n, n)
                ctx = jnp.concatenate([ctx_s[pp, rows, :] for pp in range(NP)], axis=1)
                att.append(_dot(ctx, wo_s[...]))
            for j in range(4):
                rows = pl.ds(r0 + j * n, n)
                xm = x_s[rows, :].astype(f32) + ga * att[j]
                hb = _ln(xm) * cb1 + sb
                hb_s[rows, :] = hb
                x_s[rows, :] = xm.astype(bf16)
                h1_s[pl.ds(r0 + j * n + 8, n), :] = _gelu(_dot(_ln(hb).astype(bf16), w1_s[...]))
            return carry
        jax.lax.fori_loop(0, S // RB, stage1, 0)
        cp_w2.wait()
        cp_w3.wait()
        cp_w4.wait()

        def stage2(r, carry):
            r0 = pl.multiple_of(r * RB, RB)
            n = RB // 2
            lane = jax.lax.broadcasted_iota(jnp.int32, (n, 128), 1)
            shifted, x1s, ts = [], [], []
            for j in range(2):
                hh = h1_s[pl.ds(r0 + j * n, n + 16), :]
                g0 = hh[7:7 + n, 0:256]
                g1 = hh[9:9 + n, 128:384]
                g2 = hh[6:6 + n, 256:512]
                g3 = hh[10:10 + n, 384:640]
                shifted.append(jnp.concatenate([
                    g0[:, 0:128],
                    jnp.where(lane < 32, g0[:, 128:256], g1[:, 0:128]),
                    jnp.where(lane < 64, g1[:, 128:256], g2[:, 0:128]),
                    jnp.where(lane < 96, g2[:, 128:256], g3[:, 0:128]),
                    g3[:, 128:256]], axis=1).astype(bf16))
            for j in range(2):
                x1s.append(hb_s[pl.ds(r0 + j * n, n), :] + _dot(shifted[j], w2_s[...]))
            for j in range(2):
                ts.append(_dot_nt(_ln(x1s[j]).astype(bf16), w3t_s[...]))
            for j in range(2):
                rows = pl.ds(r0 + j * n, n)
                h2 = _dot(_gelu(ts[j]).astype(bf16), w4_s[...])
                x_s[rows, :] = (x_s[rows, :].astype(f32) + gb * (x1s[j] + h2)).astype(bf16)
            rows = pl.ds(r0, RB)
            pltpu.make_async_copy(x_s.at[rows, :], o_hbm.at[rows, :], osem.at[r]).start()
            return carry
        jax.lax.fori_loop(0, S // RB, stage2, 0)
        for r in range(S // RB):
            rows = pl.ds(r * RB, RB)
            pltpu.make_async_copy(x_s.at[rows, :], o_hbm.at[rows, :], osem.at[r]).wait()


@jax.jit
def pallas_adaLN_cond__compressed_kv_cla__mixer_s_mlp__prompt_kernel(
    A_x: jax.Array,
    A_c_kv: jax.Array,
    A_w_q: jax.Array,
    A_w_uk: jax.Array,
    A_w_uv: jax.Array,
    A_w_o: jax.Array,
    B_x: jax.Array,
    B_w1: jax.Array,
    B_w2: jax.Array,
    B_w3: jax.Array,
    B_w4: jax.Array,
    c: jax.Array,
    w_mod: jax.Array,
):
    hbm = pl.BlockSpec(memory_space=pl.ANY)
    out = pl.pallas_call(
        _kernel,
        grid=(NP,),
        in_specs=[hbm] * 10 + [pl.BlockSpec((1, M), lambda p: (0, 0)), hbm],
        out_specs=hbm,
        out_shape=jax.ShapeDtypeStruct((S, M), bf16),
        scratch_shapes=[
            pltpu.VMEM((S, M), bf16),
            pltpu.VMEM((S, DC), bf16),
            pltpu.VMEM((2, M, D), u32),
            pltpu.VMEM((2, DC, D), u32),
            pltpu.VMEM((2, DC, D), u32),
            pltpu.VMEM((H * D, M), bf16),
            pltpu.VMEM((M, M), bf16),
            pltpu.VMEM((M, M), bf16),
            pltpu.VMEM((F, M), bf16),
            pltpu.VMEM((F, M), bf16),
            pltpu.VMEM((M, 6 * M), bf16),
            pltpu.VMEM((S, M), bf16),
            pltpu.VMEM((NP, S, 2 * D), bf16),
            pltpu.VMEM((S, M), f32),
            pltpu.VMEM((S + 16, M), f32),
            pltpu.SemaphoreType.DMA((9,)),
            pltpu.SemaphoreType.DMA((2, 3)),
            pltpu.SemaphoreType.DMA((S // RB,)),
        ],
        compiler_params=pltpu.CompilerParams(
            dimension_semantics=("arbitrary",), vmem_limit_bytes=120 * 1024 * 1024),
    )(A_x.reshape(S, M), A_c_kv.reshape(S, DC), A_w_q, A_w_uk, A_w_uv, A_w_o.reshape(H * D, M),
      B_w1, B_w2, B_w3.T, B_w4, c, w_mod)
    return out.reshape(1, S, M)
```

```python
import jax
import jax.numpy as jnp
import numpy as np
from jax.experimental import pallas as pl
from jax.experimental.pallas import tpu as pltpu

S = 2048
M = 640
H = 32
D = 128
DC = 512
F = 1728
NP = H // 2
BQ = 128
RB = 256
EPS = 1e-5
NT = (((1,), (1,)), ((), ()))
LOG2E = 1.4426950408889634
NEG = -1e30
f32 = jnp.float32
bf16 = jnp.bfloat16
u32 = jnp.uint32

BLOCK_ORDER = (6, 7, 13, 8, 11, 12, 15, 10, 9, 14, 4, 5, 0, 1, 2, 3)
LOOKAHEAD = (1,) * 22 + (5,) * 10


def _dot(a, b):
    return jnp.dot(a, b, preferred_element_type=f32)


def _dot_nt(a, b):
    return jax.lax.dot_general(a, b, NT, preferred_element_type=f32)


def _ln(x):
    mean = jnp.mean(x, axis=-1, keepdims=True)
    xc = x - mean
    var = jnp.mean(xc * xc, axis=-1, keepdims=True)
    return xc * jax.lax.rsqrt(var + EPS)


def _gelu(x):
    return 0.5 * x * (1.0 + jnp.tanh(0.7978845608028654 * (x + 0.044715 * (x * x * x))))


def _unpack_pair(w):
    lo = pltpu.bitcast(w << 16, f32).astype(bf16)
    hi = pltpu.bitcast(w & np.uint32(0xFFFF0000), f32).astype(bf16)
    return jnp.concatenate([lo, hi], axis=1)


def _attention_step(h, ckv, wq, wuk, wuv, store_ctx):
    k2 = _dot(ckv, wuk).astype(bf16)
    q2 = (_dot(h, wq) * (D ** -0.5 * LOG2E)).astype(bf16)
    v2 = _dot(ckv, wuv).astype(bf16)
    row = jax.lax.broadcasted_iota(jnp.int32, (BQ, BQ), 0)
    col = jax.lax.broadcasted_iota(jnp.int32, (BQ, BQ), 1)
    causal = col <= row
    units = [(g, i) for i in BLOCK_ORDER for g in range(2)]
    scores = {}

    def qk(u):
        g, i = u
        q = q2[i * BQ:(i + 1) * BQ, g * D:(g + 1) * D]
        k = k2[:, g * D:(g + 1) * D]
        s_off = _dot_nt(q, k[:i * BQ]) if i > 0 else None
        scores[u] = (s_off, _dot_nt(q, k[i * BQ:(i + 1) * BQ]))

    def softmax_pv(u):
        g, i = u
        s_off, s_d = scores.pop(u)
        v = v2[:, g * D:(g + 1) * D]
        s_d = jnp.where(causal, s_d, NEG)
        m = jnp.max(s_d, axis=1, keepdims=True)
        if i > 0:
            m = jnp.maximum(m, jnp.max(s_off, axis=1, keepdims=True))
        p_d = jnp.exp2(s_d - m)
        l = jnp.sum(p_d, axis=1, keepdims=True)
        if i > 0:
            p_off = jnp.exp2(s_off - m)
            l = l + jnp.sum(p_off, axis=1, keepdims=True)
            p_off = p_off.astype(bf16)
        o = _dot(p_d.astype(bf16), v[i * BQ:(i + 1) * BQ])
        if i > 0:
            o = o + _dot(p_off, v[:i * BQ])
        r = pl.reciprocal(l, approx=True)
        r = r * (2.0 - l * r)
        store_ctx(g, i, (o * r).astype(bf16))

    issued = 0
    for t, u in enumerate(units):
        while issued < len(units) and issued <= t + LOOKAHEAD[t]:
            qk(units[issued])
            issued += 1
        softmax_pv(u)


def _kernel(x_hbm, ckv_hbm, wq_hbm, wuk_hbm, wuv_hbm, wo_hbm, w1_hbm, w2_hbm, w3t_hbm, w4_hbm, c_ref, wmod_hbm,
            o_hbm,
            x_s, ckv_s, wq_b, wuk_b, wuv_b, wo_s, w1_s, w2_s, w3t_s, w4_s, wmod_s,
            h_s, ctx_s, hb_s, h1_s, sem, wsem, osem):
    p = pl.program_id(0)
    wq32 = wq_hbm.bitcast(u32)
    wuk32 = wuk_hbm.bitcast(u32)
    wuv32 = wuv_hbm.bitcast(u32)

    def pair_copies(pp, slot):
        return [pltpu.make_async_copy(wuk32.at[:, pp, :], wuk_b.at[slot], wsem.at[slot, 0]),
                pltpu.make_async_copy(wuv32.at[:, pp, :], wuv_b.at[slot], wsem.at[slot, 1]),
                pltpu.make_async_copy(wq32.at[:, pp, :], wq_b.at[slot], wsem.at[slot, 2])]

    cp_mod1 = pltpu.make_async_copy(wmod_hbm.at[:, 0:2 * M], wmod_s.at[:, 0:2 * M], sem.at[0])
    cp_x = pltpu.make_async_copy(x_hbm, x_s, sem.at[1])
    cp_ckv = pltpu.make_async_copy(ckv_hbm, ckv_s, sem.at[2])
    cp_wo = pltpu.make_async_copy(wo_hbm, wo_s, sem.at[3])
    cp_mod2 = pltpu.make_async_copy(wmod_hbm.at[:, 2 * M:6 * M], wmod_s.at[:, 2 * M:6 * M], sem.at[4])
    cp_w1 = pltpu.make_async_copy(w1_hbm, w1_s, sem.at[5])
    cp_w2 = pltpu.make_async_copy(w2_hbm, w2_s, sem.at[6])
    cp_w3 = pltpu.make_async_copy(w3t_hbm, w3t_s, sem.at[7])
    cp_w4 = pltpu.make_async_copy(w4_hbm, w4_s, sem.at[8])

    def silu_c():
        cc = c_ref[...].astype(f32)
        return jnp.broadcast_to(cc * jax.nn.sigmoid(cc), (8, M)).astype(bf16)

    @pl.when(p == 0)
    def _prologue():
        for cp in [cp_mod1, cp_x, cp_ckv] + pair_copies(0, 0):
            cp.start()
        sc = silu_c()
        cp_mod1.wait()
        mod = _dot(sc, wmod_s[:, 0:2 * M])
        sa = mod[0:1, 0:M]
        ca1 = 1.0 + mod[0:1, M:2 * M]
        cp_x.wait()

        def ln_chunk(r, carry):
            rows = pl.ds(pl.multiple_of(r * RB, RB), RB)
            h_s[rows, :] = (_ln(x_s[rows, :].astype(f32)) * ca1 + sa).astype(bf16)
            return carry
        jax.lax.fori_loop(0, S // RB, ln_chunk, 0)
        cp_ckv.wait()
        for cp in pair_copies(1, 1):
            cp.start()
        for cp in (cp_wo, cp_mod2, cp_w1, cp_w2, cp_w3, cp_w4):
            cp.start()

    slot = p % 2

    @pl.when(jnp.logical_and(p > 0, p + 1 < NP))
    def _prefetch():
        for cp in pair_copies(p + 1, 1 - slot):
            cp.start()

    for cp in pair_copies(p, slot):
        cp.wait()

    def store_ctx(g, i, val):
        ctx_s[p, i * BQ:(i + 1) * BQ, g * D:(g + 1) * D] = val

    _attention_step(h_s[...], ckv_s[...], _unpack_pair(wq_b[slot]), _unpack_pair(wuk_b[slot]),
                    _unpack_pair(wuv_b[slot]), store_ctx)

    @pl.when(p == NP - 1)
    def _mixer():
        cp_mod2.wait()
        mod = _dot(silu_c(), wmod_s[:, 2 * M:6 * M])
        ga = mod[0:1, 0:M]
        sb = mod[0:1, M:2 * M]
        cb1 = 1.0 + mod[0:1, 2 * M:3 * M]
        gb = mod[0:1, 3 * M:4 * M]
        cp_wo.wait()
        cp_w1.wait()
        h1_s[0:8, :] = jnp.zeros((8, M), f32)
        h1_s[S + 8:S + 16, :] = jnp.zeros((8, M), f32)

        def stage1(r, carry):
            r0 = pl.multiple_of(r * RB, RB)
            n = RB // 4
            att = []
            for j in range(4):
                rows = pl.ds(r0 + j * n, n)
                ctx = jnp.concatenate([ctx_s[pp, rows, :] for pp in range(NP)], axis=1)
                att.append(_dot(ctx, wo_s[...]))
            for j in range(4):
                rows = pl.ds(r0 + j * n, n)
                xm = x_s[rows, :].astype(f32) + ga * att[j]
                hb = _ln(xm) * cb1 + sb
                hb_s[rows, :] = hb
                x_s[rows, :] = xm.astype(bf16)
                h1_s[pl.ds(r0 + j * n + 8, n), :] = _gelu(_dot(_ln(hb).astype(bf16), w1_s[...]))
            return carry
        jax.lax.fori_loop(0, S // RB, stage1, 0)
        cp_w2.wait()
        cp_w3.wait()
        cp_w4.wait()

        def stage2(r, carry):
            r0 = pl.multiple_of(r * RB, RB)
            n = RB // 2
            lane = jax.lax.broadcasted_iota(jnp.int32, (n, 128), 1)
            shifted, x1s, ts = [], [], []
            for j in range(2):
                hh = h1_s[pl.ds(r0 + j * n, n + 16), :]
                g0 = hh[7:7 + n, 0:256]
                g1 = hh[9:9 + n, 128:384]
                g2 = hh[6:6 + n, 256:512]
                g3 = hh[10:10 + n, 384:640]
                shifted.append(jnp.concatenate([
                    g0[:, 0:128],
                    jnp.where(lane < 32, g0[:, 128:256], g1[:, 0:128]),
                    jnp.where(lane < 64, g1[:, 128:256], g2[:, 0:128]),
                    jnp.where(lane < 96, g2[:, 128:256], g3[:, 0:128]),
                    g3[:, 128:256]], axis=1).astype(bf16))
            for j in range(2):
                x1s.append(hb_s[pl.ds(r0 + j * n, n), :] + _dot(shifted[j], w2_s[...]))
            for j in range(2):
                ts.append(_dot_nt(_ln(x1s[j]).astype(bf16), w3t_s[...]))
            for j in range(2):
                rows = pl.ds(r0 + j * n, n)
                h2 = _dot(_gelu(ts[j]).astype(bf16), w4_s[...])
                x_s[rows, :] = (x_s[rows, :].astype(f32) + gb * (x1s[j] + h2)).astype(bf16)
            rows = pl.ds(r0, RB)
            pltpu.make_async_copy(x_s.at[rows, :], o_hbm.at[rows, :], osem.at[r]).start()
            return carry
        jax.lax.fori_loop(0, S // RB, stage2, 0)
        for r in range(S // RB):
            rows = pl.ds(r * RB, RB)
            pltpu.make_async_copy(x_s.at[rows, :], o_hbm.at[rows, :], osem.at[r]).wait()


@jax.jit
def pallas_adaLN_cond__compressed_kv_cla__mixer_s_mlp__prompt_kernel(
    A_x: jax.Array,
    A_c_kv: jax.Array,
    A_w_q: jax.Array,
    A_w_uk: jax.Array,
    A_w_uv: jax.Array,
    A_w_o: jax.Array,
    B_x: jax.Array,
    B_w1: jax.Array,
    B_w2: jax.Array,
    B_w3: jax.Array,
    B_w4: jax.Array,
    c: jax.Array,
    w_mod: jax.Array,
):
    hbm = pl.BlockSpec(memory_space=pl.ANY)
    out = pl.pallas_call(
        _kernel,
        grid=(NP,),
        in_specs=[hbm] * 10 + [pl.BlockSpec((1, M), lambda p: (0, 0)), hbm],
        out_specs=hbm,
        out_shape=jax.ShapeDtypeStruct((S, M), bf16),
        scratch_shapes=[
            pltpu.VMEM((S, M), bf16),
            pltpu.VMEM((S, DC), bf16),
            pltpu.VMEM((2, M, D), u32),
            pltpu.VMEM((2, DC, D), u32),
            pltpu.VMEM((2, DC, D), u32),
            pltpu.VMEM((H * D, M), bf16),
            pltpu.VMEM((M, M), bf16),
            pltpu.VMEM((M, M), bf16),
            pltpu.VMEM((F, M), bf16),
            pltpu.VMEM((F, M), bf16),
            pltpu.VMEM((M, 6 * M), bf16),
            pltpu.VMEM((S, M), bf16),
            pltpu.VMEM((NP, S, 2 * D), bf16),
            pltpu.VMEM((S, M), f32),
            pltpu.VMEM((S + 16, M), f32),
            pltpu.SemaphoreType.DMA((9,)),
            pltpu.SemaphoreType.DMA((2, 3)),
            pltpu.SemaphoreType.DMA((S // RB,)),
        ],
        compiler_params=pltpu.CompilerParams(
            dimension_semantics=("arbitrary",), vmem_limit_bytes=120 * 1024 * 1024),
    )(A_x.reshape(S, M), A_c_kv.reshape(S, DC), A_w_q, A_w_uk, A_w_uv, A_w_o.reshape(H * D, M),
      B_w1, B_w2, B_w3.T, B_w4, c, w_mod)
    return out.reshape(1, S, M)
```
